```python
import os as _os
_os.environ.setdefault("JAX_PLATFORMS", "cpu")
import jax
import jax.numpy as jnp

def _softmax(x, axis=-1):
    return jax.nn.softmax(x, axis=axis)
def _gelu(x):
    return jax.nn.gelu(x, approximate=True)
def _silu(x):
    return jax.nn.silu(x)
def _sigmoid(x):
    return jax.nn.sigmoid(x)
def _layernorm(x, axis=-1, eps=1e-5):
    m = jnp.mean(x, axis=axis, keepdims=True)
    v = jnp.var(x, axis=axis, keepdims=True)
    return (x - m) / jnp.sqrt(v + eps)
def _scatter_add(tgt, idx, src, axis=0):
    return tgt.at[idx].add(src)
def _segment_sum(src, seg, n):
    return jax.ops.segment_sum(src, seg, n)
class _Rng:
    def __init__(self, key):
        self._k = key
    def _next(self):
        self._k, sub = jax.random.split(self._k)
        return sub
    def normal(self, shape):
        return jax.random.normal(self._next(), shape, dtype=jnp.bfloat16)
    def randint(self, lo, hi, shape):
        return jax.random.randint(self._next(), shape, lo, hi, dtype=jnp.int32)
    def uniform(self, shape, lo=0.0, hi=1.0):
        return jax.random.uniform(self._next(), shape, jnp.bfloat16, lo, hi)
    def permutation(self, n):
        return jax.random.permutation(self._next(), n)


kernel_name = 'concat_heads__mha_block_cached__gqa_block_cached__near_ridge'

def setup_inputs():
    _rng = _Rng(jax.random.key(int.from_bytes(__import__("os").urandom(4), "little")))
    _w = (lambda a: (lambda t: t.astype(jnp.bfloat16) if jnp.issubdtype(t.dtype, jnp.floating) else t)(jnp.asarray(a)))
    def _A_setup():
        B, Sq, D = 8, 128, 512
        H, Sk, Dh = 32, 1024, 128
        return {
            "x": _w((lambda *s: _rng.normal(s) * 0.8)(B, Sq, D)),
            "k_cache": _w((lambda *s: _rng.normal(s) * 0.8)(B, H, Sk, Dh)),
            "v_cache": _w((lambda *s: _rng.normal(s) * 0.05)(B, H, Sk, Dh)),
            "wq": _w((lambda *s: _rng.normal(s) * 0.8)(D, H * Dh) * (D ** -0.5)),
            "wo": _w((lambda *s: _rng.normal(s) * 0.05)(H * Dh, D) * ((H * Dh) ** -0.5)),
        }
    _A_in = _A_setup()

    def _B_setup():
        B, Sq, D = 8, 128, 512
        Hq, Hkv, Sk, Dh = 32, 32, 1024, 128
        assert Hq % Hkv == 0, (Hq, Hkv)
        return {
            "x": _w((lambda *s: _rng.normal(s) * 0.8)(B, Sq, D)),
            "k_cache": _w((lambda *s: _rng.normal(s) * 0.8)(B, Hkv, Sk, Dh)),
            "v_cache": _w((lambda *s: _rng.normal(s) * 0.05)(B, Hkv, Sk, Dh)),
            "wq": _w((lambda *s: _rng.normal(s) * 0.8)(D, Hq * Dh) * (D ** -0.5)),
            "wo": _w((lambda *s: _rng.normal(s) * 0.05)(Hq * Dh, D) * ((Hq * Dh) ** -0.5)),
        }
    _B_in = _B_setup()

    return {
        "A_x": _A_in["x"],
        "A_k_cache": _A_in["k_cache"],
        "A_v_cache": _A_in["v_cache"],
        "A_wq": _A_in["wq"],
        "A_wo": _A_in["wo"],
        "B_x": _B_in["x"],
        "B_k_cache": _B_in["k_cache"],
        "B_v_cache": _B_in["v_cache"],
        "B_wq": _B_in["wq"],
        "B_wo": _B_in["wo"],
    }

def reference(A_x, A_k_cache, A_v_cache, A_wq, A_wo, B_x, B_k_cache, B_v_cache, B_wq, B_wo):
    def _A_ref(x, k_cache, v_cache, wq, wo):
        B, Sq, D = x.shape
        H, Dh = 32, 128
        q = (lambda x, *d: x.transpose(*d))((x @ wq).reshape(B, Sq, H, Dh), 0, 2, 1, 3)
        scores = jnp.einsum("bhqd,bhkd->bhqk", q, k_cache) * (Dh ** -0.5)
        p = _softmax(scores, axis=-1)
        o = jnp.einsum("bhqk,bhkd->bhqd", p, v_cache)
        return (lambda x, *d: x.transpose(*d))(o, 0, 2, 1, 3).reshape(B, Sq, H * Dh) @ wo

    def _B_ref(x, k_cache, v_cache, wq, wo):
        B, Sq, D = x.shape
        Hq, Dh = 32, 128
        Hkv = k_cache.shape[1]
        rep = Hq // Hkv
        q = (lambda x, *d: x.transpose(*d))((x @ wq).reshape(B, Sq, Hq, Dh), 0, 2, 1, 3)
        k = jnp.repeat(k_cache, rep, axis=1)
        v = jnp.repeat(v_cache, rep, axis=1)
        scores = jnp.einsum("bhqd,bhkd->bhqk", q, k) * (Dh ** -0.5)
        p = _softmax(scores, axis=-1)
        o = jnp.einsum("bhqk,bhkd->bhqd", p, v)
        return (lambda x, *d: x.transpose(*d))(o, 0, 2, 1, 3).reshape(B, Sq, Hq * Dh) @ wo

    a = _A_ref(A_x, A_k_cache, A_v_cache, A_wq, A_wo)
    b = _B_ref(B_x, B_k_cache, B_v_cache, B_wq, B_wo)
    return jnp.concatenate([a, b], axis=-1)
```

```python
import jax
import jax.numpy as jnp
from jax import lax
import jax.experimental.pallas as pl
import jax.experimental.pallas.tpu as pltpu

RING = 4
WCH = 4
G = 8
GT = 2
LOG2E = 1.4426950408889634


@jax.jit
def pallas_concat_heads__mha_block_cached__gqa_block_cached__near_ridge_kernel(
        A_x, A_k_cache, A_v_cache, A_wq, A_wo, B_x, B_k_cache, B_v_cache, B_wq, B_wo):
    B, Sq, D = A_x.shape
    _, H, Sk, Dh = A_k_cache.shape
    M = B * Sq
    HC = H // WCH
    c = (Dh ** -0.5) * LOG2E
    A_x = A_x.reshape(M, D)
    B_x = B_x.reshape(M, D)

    def kernel(ax, ak, av, awq, awo, bx, bk, bv, bwq, bwo, out,
               xb, kb, vb, wqb, wob, qb, ob, acc, outb, xs, ks, vs, wqs, wos, os_, ts):
        X, K, V, WQ, WO = (ax, bx), (ak, bk), (av, bv), (awq, bwq), (awo, bwo)

        def x_cp(br):
            return pltpu.make_async_copy(X[br], xb.at[br], xs.at[br])

        def wq_cp(br, j):
            off = j * (HC * Dh)
            if not isinstance(j, int):
                off = pl.multiple_of(off, HC * Dh)
            return pltpu.make_async_copy(WQ[br].at[:, pl.ds(off, HC * Dh)],
                                         wqb.at[br, :, pl.ds(off, HC * Dh)], wqs.at[br, j])

        def wo_cp(br, j):
            off = j * (HC * Dh)
            if not isinstance(j, int):
                off = pl.multiple_of(off, HC * Dh)
            return pltpu.make_async_copy(WO[br].at[pl.ds(off, HC * Dh), :],
                                         wob.at[br, pl.ds(off, HC * Dh), :], wos.at[br, j])

        def k_cp(br, h, b):
            s = h % RING
            return pltpu.make_async_copy(K[br].at[b, h], kb.at[s, b], ks.at[s, b])

        def v_cp(br, h, b):
            s = h % RING
            return pltpu.make_async_copy(V[br].at[b, h], vb.at[s, b], vs.at[s, b])

        def out_cp(br):
            return pltpu.make_async_copy(outb.at[br], out.at[:, pl.ds(br * D, D)], os_.at[br])

        def tail_cp(g):
            rows = pl.ds(g * GT * Sq, GT * Sq)
            return pltpu.make_async_copy(outb.at[1, rows], out.at[rows, pl.ds(D, D)], ts.at[g])

        def attend(s_, b):
            s = lax.dot_general(qb[b * Sq:(b + 1) * Sq, :], kb[s_, b],
                                (((1,), (1,)), ((), ())), preferred_element_type=jnp.float32)
            m = jnp.max(s, axis=-1, keepdims=True)
            p = jnp.exp2(s - m)
            l = jnp.sum(p, axis=-1, keepdims=True)
            o = jnp.dot(p.astype(jnp.bfloat16), vb[s_, b], preferred_element_type=jnp.float32)
            ob[b * Sq:(b + 1) * Sq, :] = (o * (1.0 / l)).astype(jnp.bfloat16)

        x_cp(0).start()
        wq_cp(0, 0).start()
        for h in range(RING):
            for b in range(B):
                k_cp(0, h, b).start()
                v_cp(0, h, b).start()
            if h == 0:
                wo_cp(0, 0).start()
                x_cp(1).start()

        for br in range(2):
            x_cp(br).wait()
            acc[...] = jnp.zeros_like(acc)

            def head(h, carry, br=br):
                j = h // HC

                @pl.when(h % HC == 0)
                def _():
                    wq_cp(br, j).wait()

                    @pl.when(j + 1 < WCH)
                    def _():
                        wq_cp(br, j + 1).start()
                        wo_cp(br, j + 1).start()
                    if br == 0:
                        @pl.when(j + 1 == WCH)
                        def _():
                            wq_cp(1, 0).start()
                            wo_cp(1, 0).start()

                off = pl.multiple_of(h * Dh, Dh)
                s_ = h % RING
                q = jnp.dot(xb[br], wqb[br, :, pl.ds(off, Dh)], preferred_element_type=jnp.float32)
                qb[...] = (q * c).astype(jnp.bfloat16)
                for b in range(B):
                    if b % G == 0:
                        for bb in range(b, b + G):
                            k_cp(br, h, bb).wait()
                            v_cp(br, h, bb).wait()
                    attend(s_, b)

                @pl.when(h + RING < H)
                def _():
                    for b in range(B):
                        k_cp(br, h + RING, b).start()
                        v_cp(br, h + RING, b).start()
                if br == 0:
                    @pl.when(h + RING >= H)
                    def _():
                        for b in range(B):
                            k_cp(1, h + RING - H, b).start()
                            v_cp(1, h + RING - H, b).start()

                @pl.when(h % HC == 0)
                def _():
                    wo_cp(br, j).wait()
                acc[...] += jnp.dot(ob[...], wob[br, pl.ds(off, Dh), :], preferred_element_type=jnp.float32)
                return carry

            if br == 0:
                lax.fori_loop(0, H, head, 0)
                outb[br] = acc[...].astype(outb.dtype)
                out_cp(br).start()
            else:
                lax.fori_loop(0, H - 1, head, 0)
                h = H - 1
                s_ = h % RING
                off = h * Dh
                q = jnp.dot(xb[br], wqb[br, :, off:off + Dh], preferred_element_type=jnp.float32)
                qb[...] = (q * c).astype(jnp.bfloat16)
                for g in range(B // GT):
                    for b in range(g * GT, (g + 1) * GT):
                        k_cp(br, h, b).wait()
                        v_cp(br, h, b).wait()
                    for b in range(g * GT, (g + 1) * GT):
                        attend(s_, b)
                    rows = slice(g * GT * Sq, (g + 1) * GT * Sq)
                    y = acc[rows, :] + jnp.dot(ob[rows, :], wob[br, off:off + Dh, :],
                                               preferred_element_type=jnp.float32)
                    outb[br, rows, :] = y.astype(outb.dtype)
                    tail_cp(g).start()
        out_cp(0).wait()
        for g in range(B // GT):
            tail_cp(g).wait()

    anyspec = pl.BlockSpec(memory_space=pl.ANY)
    bf = jnp.bfloat16
    res = pl.pallas_call(
        kernel,
        in_specs=[anyspec] * 10,
        out_specs=anyspec,
        out_shape=jax.ShapeDtypeStruct((M, 2 * D), bf),
        scratch_shapes=[
            pltpu.VMEM((2, M, D), bf), pltpu.VMEM((RING, B, Sk, Dh), bf), pltpu.VMEM((RING, B, Sk, Dh), bf),
            pltpu.VMEM((2, D, H * Dh), bf), pltpu.VMEM((2, H * Dh, D), bf),
            pltpu.VMEM((M, Dh), bf), pltpu.VMEM((M, Dh), bf), pltpu.VMEM((M, D), jnp.float32),
            pltpu.VMEM((2, M, D), bf),
            pltpu.SemaphoreType.DMA((2,)), pltpu.SemaphoreType.DMA((RING, B)), pltpu.SemaphoreType.DMA((RING, B)),
            pltpu.SemaphoreType.DMA((2, WCH)), pltpu.SemaphoreType.DMA((2, WCH)), pltpu.SemaphoreType.DMA((2,)),
            pltpu.SemaphoreType.DMA((B // GT,)),
        ],
        compiler_params=pltpu.CompilerParams(vmem_limit_bytes=100 * 1024 * 1024),
    )(A_x, A_k_cache, A_v_cache, A_wq, A_wo, B_x, B_k_cache, B_v_cache, B_wq, B_wo)
    return res.reshape(B, Sq, 2 * D)
```
